```python
import jax
import jax.numpy as jnp

def _softmax(x, axis=-1):
    return jax.nn.softmax(x, axis=axis)
def _gelu(x):
    return jax.nn.gelu(x, approximate=True)
def _silu(x):
    return jax.nn.silu(x)
def _sigmoid(x):
    return jax.nn.sigmoid(x)
def _layernorm(x, axis=-1, eps=1e-5):
    m = jnp.mean(x, axis=axis, keepdims=True)
    v = jnp.var(x, axis=axis, keepdims=True)
    return (x - m) / jnp.sqrt(v + eps)
def _scatter_add(tgt, idx, src, axis=0):
    return tgt.at[idx].add(src)
def _segment_sum(src, seg, n):
    return jax.ops.segment_sum(src, seg, n)
class _Rng:
    def __init__(self, key):
        self._k = key
    def _next(self):
        self._k, sub = jax.random.split(self._k)
        return sub
    def normal(self, shape):
        return jax.random.normal(self._next(), shape, dtype=jnp.bfloat16)
    def randint(self, lo, hi, shape):
        return jax.random.randint(self._next(), shape, lo, hi, dtype=jnp.int32)
    def uniform(self, shape, lo=0.0, hi=1.0):
        return jax.random.uniform(self._next(), shape, jnp.bfloat16, lo, hi)
    def permutation(self, n):
        return jax.random.permutation(self._next(), n)


kernel_name = 'parallel_sum__sliding_local_dilated__mixer_channel_mlp__prompt'

def _fwd_setup_inputs():
    _rng = _Rng(jax.random.key(int.from_bytes(__import__("os").urandom(4), "little")))
    _w = (lambda a: (lambda t: t.astype(jnp.bfloat16) if jnp.issubdtype(t.dtype, jnp.floating) else t)(jnp.asarray(a)))
    def _A_setup():
        B, S, D = 1, 2048, 576
        return {
            "x": _w((lambda *s: _rng.normal(s) * 0.05)(B, S, D)),
            "wqkv": _w((lambda *s: _rng.normal(s) * 0.05)(D, 3 * D)),
            "wo": _w((lambda *s: _rng.normal(s) * 0.05)(D, D)),
        }
    _A_in = _A_setup()

    def _B_setup():
        B, S, D, F = 1, 2048, 576, 4608
        return {
            "x": _w((lambda *s: _rng.normal(s) * 0.05)(B, S, D)),
            "w1": _w((lambda *s: _rng.normal(s) * 0.05)(D, F) * (D ** -0.5)),
            "b1": _w((lambda *s: _rng.normal(s) * 0.05)(F)),
            "w2": _w((lambda *s: _rng.normal(s) * 0.05)(F, D) * (F ** -0.5)),
            "b2": _w((lambda *s: _rng.normal(s) * 0.05)(D)),
        }
    _B_in = _B_setup()

    return {
        "A_x": _A_in["x"],
        "A_wqkv": _A_in["wqkv"],
        "A_wo": _A_in["wo"],
        "B_x": _B_in["x"],
        "B_w1": _B_in["w1"],
        "B_b1": _B_in["b1"],
        "B_w2": _B_in["w2"],
        "B_b2": _B_in["b2"],
    }

def _fwd_reference(A_x, A_wqkv, A_wo, B_x, B_w1, B_b1, B_w2, B_b2):
    def _A_ref(x, wqkv, wo):
        B, S, D = x.shape
        H = 32; Dh = D // H
        W, dil = 8, 2
        qkv = (lambda x, *d: x.transpose(*d))((x @ wqkv).reshape(B, S, 3, H, Dh), 2, 0, 3, 1, 4)
        q, k, v = qkv[0], qkv[1], qkv[2]
        scale = Dh ** -0.5
        pos = jnp.arange(S)
        off = jnp.arange(W) * dil
        idx = pos[:, None] - off[None, :]
        mask = idx >= 0
        idx_c = jnp.where(mask, idx, 0).reshape(-1)
        kg = k[:, :, idx_c, :].reshape(B, H, S, W, Dh)
        vg = v[:, :, idx_c, :].reshape(B, H, S, W, Dh)
        logits = jnp.einsum("bhsd,bhswd->bhsw", q, kg) * scale
        logits = jnp.where(mask[None, None, :, :], logits, -1e9)
        attn = _softmax(logits, axis=-1)
        o = jnp.einsum("bhsw,bhswd->bhsd", attn, vg)
        return (lambda x, *d: x.transpose(*d))(o, 0, 2, 1, 3).reshape(B, S, D) @ wo

    def _B_ref(x, w1, b1, w2, b2):
        y = _layernorm(x, axis=-1)
        h = _gelu(jnp.einsum("bsd,df->bsf", y, w1) + b1)
        return jnp.einsum("bsf,fd->bsd", h, w2) + b2

    x = A_x
    xn = _layernorm(x, axis=-1)
    return x + _A_ref(xn, A_wqkv, A_wo) + _B_ref(xn, B_w1, B_b1, B_w2, B_b2)


def setup_inputs():
    _inp = _fwd_setup_inputs()
    _gk = jax.random.fold_in(jax.random.key(int.from_bytes(__import__("os").urandom(4), "little")), 2**31 - 1)
    _shapes = [[1, 2048, 576]]
    _dtypes = ['bfloat16']
    _gks = jax.random.split(_gk, len(_shapes))
    _gs = [jax.random.normal(k, s, dtype=jnp.dtype(d)) * 0.05 for k, s, d in zip(_gks, _shapes, _dtypes)]
    _inp["grad_out"] = _gs[0]
    return _inp

def reference(A_x, A_wqkv, A_wo, B_w1, B_b1, B_w2, B_b2, B_x, grad_out):
    _const = dict(B_x=B_x)
    def _f(*_d):
        return _fwd_reference(**{'A_x': _d[0], 'A_wqkv': _d[1], 'A_wo': _d[2], 'B_w1': _d[3], 'B_b1': _d[4], 'B_w2': _d[5], 'B_b2': _d[6], **_const})
    _out, _vjp = jax.vjp(_f, A_x, A_wqkv, A_wo, B_w1, B_b1, B_w2, B_b2)
    _grads = _vjp(grad_out)
    _out0 = jnp.asarray(_out)
    return (_out0, *[jnp.asarray(_g) for _g in _grads])
```

```python
import functools

import jax
import jax.numpy as jnp
from jax import lax
from jax.experimental import pallas as pl
from jax.experimental.pallas import tpu as pltpu

S, D, F = 2048, 576, 4608
DH, WIN, DIL = 18, 8, 2
DP = 640
DM = 512
Q3 = 3 * D
FC = 512
NC = F // FC
HS = S // 2
HG = 8 * DH
EPS = 1e-5
LP = 1
LB = 1
ATT_SPLIT = (3, 15, 45, 75)
IDLE = (6, 30, 14)
NB = 4

F32, BF16, U32 = jnp.float32, jnp.bfloat16, jnp.uint32
NN = (((1,), (0,)), ((), ()))
NT = (((1,), (1,)), ((), ()))


def _dot(a, b, dims=NN):
    return lax.dot_general(a, b, dims, preferred_element_type=F32)


class _Grid:
    def __init__(self, rows):
        self.rows = rows

    def __add__(self, o):
        return _Grid([[a + b for a, b in zip(r, s)] for r, s in zip(self.rows, o.rows)])

    def __sub__(self, o):
        return _Grid([[a - b for a, b in zip(r, s)] for r, s in zip(self.rows, o.rows)])

    def quadrants(self):
        n = len(self.rows) // 2
        return [_Grid([r[j * n:(j + 1) * n] for r in self.rows[i * n:(i + 1) * n]])
                for i in range(2) for j in range(2)]


def _lhs_forms(a11, a12, a21, a22):
    return [a11 + a22, a21 + a22, a11, a22, a11 + a12, a21 - a11, a12 - a22]


def _rhs_forms(b11, b12, b21, b22):
    return [b11 + b22, b11, b12 - b22, b21 - b11, b22, b11 + b12, b21 + b22]


def _cot_forms(g11, g12, g21, g22):
    return [g11 + g22, g21 - g22, g12 + g22, g11 + g21, g12 - g11, g22, g11]


def _out_sums(m1, m2, m3, m4, m5, m6, m7):
    return [m1 + m4 - m5 + m7, m3 + m5, m2 + m4, m1 - m2 + m3 + m6]


def _lhs_sums(n1, n2, n3, n4, n5, n6, n7):
    return [n1 + n3 + n5 - n6, n5 + n7, n2 + n6, n1 + n2 + n4 - n7]


def _expand(forms, rows):
    if len(rows) == 1:
        return [rows[0][0]]
    return [x for g in forms(*_Grid(rows).quadrants()) for x in _expand(forms, g.rows)]


def _collapse(sums, prods):
    if len(prods) == 1:
        return [[prods[0]]]
    n = len(prods) // 7
    c11, c12, c21, c22 = sums(*[_Grid(_collapse(sums, prods[i * n:(i + 1) * n])) for i in range(7)])
    return ([r + s for r, s in zip(c11.rows, c12.rows)] + [r + s for r, s in zip(c21.rows, c22.rows)])


def _pack(even, odd):
    return pltpu.pack_elementwise([even, odd], packed_dtype=BF16)


class _Packed:
    def __init__(self, ref):
        self.ref = ref

    def get(self, lead, row, nrows, lanes, gate=None):
        words = self.ref[(*lead, _rows(row >> 1, nrows // 2), lanes)]
        return pltpu.bitcast(gate(words) if gate else words, BF16)

    def put(self, lead, row, lanes, value):
        self.put_words(lead, row, lanes, pltpu.bitcast(value.astype(BF16), U32))

    def put_pair(self, lead, row, lanes, even, odd):
        return self.put_words(lead, row, lanes, _pack(even, odd))

    def put_words(self, lead, row, lanes, words):
        self.ref[(*lead, _rows(row >> 1, words.shape[0]), lanes)] = words
        return words


def _packed(*shape):
    return pltpu.VMEM((*shape[:-2], shape[-2] // 2, shape[-1]), U32)


def _rows(start, size):
    return pl.ds(start if isinstance(start, int) else pl.multiple_of(start, 8), size)


class _Pacer:
    def __init__(self, zero):
        self.never = jnp.zeros((8, 128), jnp.int32) + zero

    def gate(self, token):
        def apply(x):
            reps = (x.shape[0] // 8, x.shape[1] // 128)
            t = token if token.dtype == x.dtype else pltpu.bitcast(token, x.dtype)
            return jnp.where(jnp.tile(self.never, reps) != 0, jnp.tile(t, reps), x)
        return apply

    def run(self, dots, *sides):
        done = [0] * len(sides)
        for k, dot in enumerate(dots):
            result = dot()
            tasks = []
            for n, side in enumerate(sides):
                upto = (k + 1) * len(side) // len(dots)
                tasks += [((m + 0.5) / (upto - done[n]), n, t) for m, t in enumerate(side[done[n]:upto])]
                done[n] = upto
            tasks = [t for _, _, t in sorted(tasks, key=lambda e: e[:2])]
            for n, task in enumerate(tasks):
                row = result.shape[0] // 8 * n // len(tasks) * 8
                task(self.gate(result[row:row + 8, :128]))


def _gelu_and_grad(u):
    c0 = 0.7978845608028654
    c1 = c0 * 0.044715
    u2 = u * u
    t = jnp.tanh(u * (c0 + c1 * u2))
    cdf = 0.5 + 0.5 * t
    return u * cdf, cdf + (u * (0.5 * c0 + (1.5 * c1) * u2)) * (1.0 - t * t)


def _idle(gate):
    return None


def _colmean(a):
    return jnp.sum(a, axis=0, keepdims=True) * (1.0 / D)


def _sum(terms):
    acc = terms[0]
    for t in terms[1:]:
        acc = acc + t
    return acc


def _kernel(x_hbm, wqkv_hbm, wo_hbm, w1_hbm, b1_ref, w2_hbm, b2_ref, g_hbm,
            out_hbm, dx_hbm, dwqkv_hbm, dwo_hbm, dw1_hbm, db1_ref, dw2_hbm, db2_ref,
            x_v, g_v, xn_v, xnb, stats, dqkv, o_v, wqkv_v, wot, acc_o, acc_y, sems):
    np_, nb_ = 2 ** LP, 2 ** LB
    rp, rb = 7 ** LP, 7 ** LB
    part = functools.partial
    xnb, dqkv, o_v, wot = map(_Packed, (xnb, dqkv, o_v, wot))

    word = pltpu.bitcast(b2_ref[:, pl.ds(0, 128)].astype(F32), jnp.int32)[0, 0]
    opaque_zero = (word * (word + 1)) & 1

    pacer = _Pacer(opaque_zero)
    z = opaque_zero

    def cols(t, n=128):
        return pl.ds(t if isinstance(t, int) else pl.multiple_of(t, 128), n)

    def padded_rows(t, fill=None):
        if fill is None:
            return jnp.concatenate([t, jnp.zeros_like(t)], axis=0)
        row = lax.broadcasted_iota(jnp.int32, t.shape, 0)
        return jnp.concatenate([t, jnp.where(row == 0, fill, 0.0)], axis=0)

    def main(qkv, do_v, rhs_y, rhs_g, rem_y, cot_y, cot_g, w1_buf, w2_buf,
             lhs_pre, lhs_dh, rem_pre, rem_dh, wt):
        qkv, do_v, rhs_y, rhs_g, rem_y, cot_y, cot_g, lhs_pre, lhs_dh, rem_pre, rem_dh = map(
            _Packed, (qkv, do_v, rhs_y, rhs_g, rem_y, cot_y, cot_g, lhs_pre, lhs_dh, rem_pre, rem_dh))

        def chunk_cols(c):
            return pl.ds(c * FC if isinstance(c, int) else pl.multiple_of(c * FC, FC), FC)

        def w_copies(c, slot):
            chunk = chunk_cols(c)
            return (pltpu.make_async_copy(w1_hbm.at[:, chunk], w1_buf.at[slot], sems.at[0]),
                    pltpu.make_async_copy(w2_hbm.at[:, chunk], w2_buf.at[slot], sems.at[1]))

        def rhs_stack_tasks(src, rhs, t0):
            kq, tq = DM // np_, S // np_

            def task(r, t, gate):
                blocks = [[gate(src[pl.ds(a * kq + r, 16), cols(b * tq + t)].astype(F32))
                           for b in range(np_)] for a in range(np_)]
                for i, v in enumerate(_expand(_rhs_forms, blocks)):
                    rhs.put((i,), r, cols(t), v)
            return [part(task, r, t) for t in (t0, t0 + 128) for r in range(0, kq, 16)]

        def cot_stack_tasks(src, cot, t0):
            mq, tq = D // nb_, S // nb_

            def task(r, t, gate):
                blocks = [[gate(src[pl.ds(a * mq + r, 16), cols(b * tq + t)].astype(F32))
                           for b in range(nb_)] for a in range(nb_)]
                for i, v in enumerate(_expand(_cot_forms, blocks)):
                    cot.put((i,), r, cols(t), v)
            return [part(task, r, t) for t in (t0, t0 + 128) for r in range(0, mq, 16)]

        def d_stack_tasks(c, slot):
            mq, kq = FC // np_, DM // np_

            def transpose(w, k, n, biased, gate):
                if k < 4:
                    v = w[slot, pl.ds(k * 128, 128), cols(n)].astype(F32)
                else:
                    fill = b1_ref[c][:, n:n + 128].astype(F32) if biased else None
                    v = padded_rows(w[slot, pl.ds(DM, 64), cols(n)].astype(F32), fill)
                v = jnp.concatenate([gate(v[:8]), v[8:]], axis=0).T
                wt[k, pl.ds(n, 128), :] = v
                return v

            def alternate(k, r, half):
                return [wt[k + z, pl.ds(r + half + 2 * m, 8, stride=4), :] for m in range(2)]

            def forms(dst, r, half, k, gate):
                blocks = [[list(map(gate, alternate(b * kq // 128 + k, a * mq + r, half))) for b in range(np_)]
                          for a in range(np_)]
                even, odd = (_expand(_lhs_forms, [[v[m] for v in row] for row in blocks]) for m in range(2))
                return [dst.put_pair((i,), r + 16 * half, cols(k * 128), even[i], odd[i]) for i in range(rp)][-1]

            def tail(rem, r, half, gate):
                for a in range(np_):
                    even, odd = alternate(4, a * mq + r, half)
                    rem.put_pair((), a * mq + r + 16 * half, slice(None), gate(even), odd)

            tasks = []
            for w, dst, rem, biased in ((w1_buf, lhs_pre, rem_pre, True), (w2_buf, lhs_dh, rem_dh, False)):
                for k in range(5):
                    for n in range(0, FC, 128):
                        tasks += [part(transpose, w, k, n, biased), _idle, _idle]
                for r in range(0, mq, 32):
                    for half in range(2):
                        tasks += [part(forms, dst, r, half, k) for k in range(kq // 128)]
                        tasks += [part(tail, rem, r, half)]
            return tasks

        def prologue(y_v, wqkvt, wo_v):
            wqkvt = _Packed(wqkvt)
            nblk = 4
            bw = S // nblk
            cp_g = [pltpu.make_async_copy(g_hbm.at[:, cols(k * bw, bw)],
                                          g_v.at[pl.ds(0, D), cols(k * bw, bw)], sems.at[2 + k])
                    for k in range(nblk)]
            cp_wo = pltpu.make_async_copy(wo_hbm, wo_v, sems.at[6])
            cp_x = pltpu.make_async_copy(x_hbm, x_v, sems.at[7])
            cp_wq = pltpu.make_async_copy(wqkv_hbm, wqkv_v, sems.at[8])
            for cp in [cp_wo] + cp_g + [cp_x, cp_wq, *w_copies(0, 0)]:
                cp.start()
            g_v[pl.ds(D, DP - D), :] = jnp.zeros((DP - D, S), BF16)
            xnb.put((), D, slice(None), jnp.zeros((DP - D, S), F32))
            cp_wo.wait()

            def zero(acc, i, t, gate):
                acc[i, t] = jnp.tile(gate(jnp.zeros((8, 128), F32)), (acc.shape[2] // 8, 1))

            def do_dot(t):
                if t % bw == 0:
                    cp_g[t // bw].wait()
                v = _dot(wo_v[...], g_v[pl.ds(0, D), cols(t, 256)])
                do_v.put((), 0, cols(t, 256), v)
                return v

            def wo_transpose(k, gate):
                n = min(128, D - k * 128)
                t = wo_v[pl.ds(k * 128, n), :].astype(F32)
                if n < 128:
                    t = padded_rows(t, b2_ref[...].astype(F32))
                wot.put((), 0, cols(k * 128), t.T)

            pacer.run([part(do_dot, t) for t in range(0, S, 256)],
                        [part(zero, acc, i, t) for acc in (acc_o, acc_y) for i in range(rb)
                       for t in range(acc.shape[1])],
                        [part(wo_transpose, k) for k in range(5)])
            cp_x.wait()
            cp_wq.wait()

            def norm(t, gate):
                v = x_v[:, cols(t)].astype(F32)
                v = jnp.concatenate([gate(v[:8]), v[8:]], axis=0)
                xc = v - _colmean(v)
                r1 = 1.0 / jnp.sqrt(_colmean(xc * xc) + EPS)
                xn = xc * r1
                m2 = _colmean(xn)
                yc = xn - m2
                r2 = 1.0 / jnp.sqrt(_colmean(yc * yc) + EPS)
                y = yc * r2
                xn_v[:, cols(t)] = xn
                xnb.put((), 0, cols(t), xn)
                y_v[:, cols(t)] = y
                rem_y.put((), 0, cols(t), padded_rows(y[DM:], 1.0))
                stats[pl.ds(0, 1), cols(t)] = r1
                stats[pl.ds(1, 1), cols(t)] = m2
                stats[pl.ds(2, 1), cols(t)] = r2

            def wqkv_transpose(q, k, gate):
                n = min(128, D - k * 128)
                t = wqkv_v[pl.ds(k * 128, n), :].astype(F32)[:, q:q + D]
                if n < 128:
                    t = padded_rows(t)
                wqkvt.put((), q, cols(k * 128), t.T)

            def bias2_grad(r, gate):
                n = min(128, D - r)
                tot = _sum([gate(g_v[pl.ds(r, 128), cols(t)].astype(F32)) for t in range(0, S, 128)])
                db2_ref[:, pl.ds(r, n)] = jnp.sum(tot.T, axis=0, keepdims=True)[:, :n].astype(BF16)

            def qkv_dot(q, t):
                v = _dot(wqkvt.get((), q + 2 * z, D, slice(None)), xnb.get((), 2 * z, DP, cols(t, 256)))
                qkv.put((), q, cols(t, 256), v)
                return v

            for k in range(5):
                wqkv_transpose(0, k, None)
            norm(0, lambda v: v)
            norm(128, lambda v: v)
            pacer.run([part(qkv_dot, 0, t) for t in range(0, S, 256)],
                        [part(norm, t) for t in range(256, S, 128)] + [_idle] * 2,
                        [part(wqkv_transpose, q, k) for q in (D, 2 * D) for k in range(5)])
            for cp in w_copies(0, 0):
                cp.wait()

            @pl.loop(0, 4)
            def _(n):
                t0 = n * 256
                pacer.run([part(qkv_dot, q, h + t0) for q in (D, 2 * D) for h in (0, HS)],
                          rhs_stack_tasks(y_v, rhs_y, t0) + cot_stack_tasks(y_v, cot_y, t0),
                          rhs_stack_tasks(g_v, rhs_g, t0) + cot_stack_tasks(g_v, cot_g, t0))

            for task in d_stack_tasks(0, 0) + [part(bias2_grad, r) for r in range(0, D, 128)]:
                task(lambda v: v)

        pl.run_scoped(prologue, pltpu.VMEM((D, S), F32), _packed(Q3, DP),
                      pltpu.VMEM((D, D), BF16))

        def loop(lhs_out, lhs_dy, dw1_st, dw2_st, a_in, a_out, ksh, vsh, pw, ds,
                 carry, db1_acc, db1_tmp, prod_a, prod_b, tail_a, tail_b, wg2, wg1, *stacks):
            lhs_out, lhs_dy, *stacks = map(_Packed, (lhs_out, lhs_dy, *stacks))
            h_st, dp_st = stacks[:NB], stacks[NB:]

            def f_stack_tasks(slot):
                mq, kq = D // nb_, FC // nb_

                def forms(src, dst, r, gate):
                    blocks = [[src[slot, pl.ds(a * mq + r, 16), pl.ds(b * kq, kq)].astype(F32)
                               for b in range(nb_)] for a in range(nb_)]
                    lo, hi = (_expand(_lhs_forms, [[gate(v[k:k + 8]) for v in row] for row in blocks])
                              for k in (0, 8))
                    for i in range(rb):
                        dst.put_pair((i,), r, slice(None), lo[i], hi[i])
                return [part(forms, src, dst, r) for src, dst in ((w2_buf, lhs_out), (w1_buf, lhs_dy))
                        for r in range(0, mq, 16)]

            def attention_tasks(c):
                piece = jnp.minimum(c, 7)
                late = 1 - piece % 2
                base = (piece // 2) * HG
                t0 = late * HS
                scale = DH ** -0.5

                lanes = lax.broadcasted_iota(jnp.int32, (8, 128), 1)

                def head_rows(d):
                    return pl.ds(d, 8, stride=DH)

                def load(w, j, r, gate):
                    src, row = (qkv, w * D + base) if w < 3 else (do_v, base)
                    t = jnp.clip(t0 + (j - (w in (1, 2))) * 128, 0, S - 128)
                    a_in[w, j, pl.ds(r, 48), :] = src.get(
                        (), row + r, 48, cols(pl.multiple_of(t, 128)), gate).astype(F32)

                def window_dots(src, other, shifted, j, lo, hi, acc, gate):
                    lane = gate(lanes)
                    for d in range(lo, hi):
                        a = gate(a_in[src + z, j, head_rows(d), :])
                        cur = a_in[other + z, j + 1, head_rows(d), :]
                        prev = a_in[other + z, j, head_rows(d), :]
                        for w in range(WIN):
                            if w:
                                b = pltpu.roll(jnp.where(lane >= 128 - DIL * w, prev, cur), DIL * w, 1)
                            else:
                                b = cur
                            shifted[d, w] = b
                            acc[w] = a * b if d == 0 else acc[w] + a * b
                    return acc[WIN - 1]

                def softmax(j, acc, gate):
                    lg = [v * scale for v in acc]
                    if j == 0:
                        lg = [jnp.where(lanes + t0 < DIL * w, -1e9, v) for w, v in enumerate(lg)]
                    top = functools.reduce(jnp.maximum, lg)
                    e = [jnp.exp(v - top) for v in lg]
                    inv = 1.0 / _sum(e)
                    for w in range(WIN):
                        pw[j, w] = e[w] * inv
                    return inv

                def softmax_grad(j, dp, gate):
                    prob = [pw[j + z, w] for w in range(WIN)]
                    mean = _sum([prob[w] * dp[w] for w in range(WIN)])
                    for w in range(WIN):
                        ds[j, w] = prob[w] * (dp[w] - mean) * scale
                    return mean

                def mix(coef, shifted, dst, j, lo, hi, gate):
                    cf = [gate(coef[j + z, w]) for w in range(WIN)]
                    for d in range(lo, hi):
                        v = _sum([cf[w] * shifted[d + z, w] for w in range(WIN)])
                        a_out[dst, j, head_rows(d), :] = v
                    return v

                def shift_back(k, coef, j, gate):
                    for w in range(WIN):
                        cur = coef[j + z, w]
                        if j == 0:
                            carry[late, k, w] = cur
                        if w:
                            nxt = coef[j + 1 + z, w] if j < 7 else jnp.where(late == 0, carry[1 + z, k, w], 0.0)
                            coef[j, w] = pltpu.roll(jnp.where(lanes < DIL * w, nxt, gate(cur)), 128 - DIL * w, 1)

                def scatter(coef, src, dst, j, lo, hi, gate):
                    lane = gate(lanes)
                    cf = [coef[j + z, w] for w in range(WIN)]
                    for d in range(lo, hi):
                        cur = gate(a_in[src + z, j, head_rows(d), :])
                        nxt = a_in[src + z, j + 1, head_rows(d), :]
                        a_out[dst, j, head_rows(d), :] = _sum([cf[0] * cur] + [
                            cf[w] * pltpu.roll(jnp.where(lane < DIL * w, nxt, cur), 128 - DIL * w, 1)
                            for w in range(1, WIN)])

                def store(w, j, r, gate):
                    dst, row = (dqkv, w * D + base) if w < 3 else (o_v, base)
                    even, odd = (a_out[w + z, j, pl.ds(r + k, 24, stride=2), :] for k in range(2))
                    dst.put_pair((), row + r, cols(pl.multiple_of(t0 + j * 128, 128)), gate(even), odd)

                def merged(main, extra):
                    order = [((n + 0.5) / len(main), t) for n, t in enumerate(main)]
                    order += [((n + 0.5) / len(extra), t) for n, t in enumerate(extra)]
                    return [t for _, t in sorted(order, key=lambda e: e[0])]

                def loads(j):
                    return [part(load, w, j, r) for w in range(4) for r in range(0, HG, 48)]

                def stores(ws, j):
                    return [part(store, w, j, r) for w in ws for r in range(0, HG, 48)]

                tasks = loads(0) + loads(1)
                for j in range(8):
                    lg, dp = [None] * WIN, [None] * WIN
                    work = [part(window_dots, 0, 1, ksh, j, d, d + 1, lg) for d in range(DH)]
                    work += [part(softmax, j, lg), _idle]
                    work += [part(window_dots, 3, 2, vsh, j, d, d + 1, dp) for d in range(DH)]
                    work += [part(softmax_grad, j, dp), _idle]
                    mixes = [part(mix, pw, vsh, 3, j, d, d + 2) for d in range(0, DH, 2)]
                    mixes += [part(mix, ds, ksh, 0, j, d, d + 2) for d in range(0, DH, 2)]
                    extra = loads(j + 2) if j < 7 else []
                    tasks += work + (merged(mixes, extra) if extra else mixes) + stores((3, 0), j)
                    for m in ([j - 1] if j else []) + ([7] if j == 7 else []):
                        tasks += [part(shift_back, k, coef, m) for k, coef in enumerate((ds, pw))] + [_idle]
                        for d in range(0, DH, 2):
                            tasks += [part(scatter, ds, 0, 1, m, d, d + 2), _idle,
                                      part(scatter, pw, 3, 2, m, d, d + 2), _idle]
                        tasks += stores((1, 2), m)
                return tasks

            def out_copies(c):
                return (pltpu.make_async_copy(dw1_st.at[c % 2], dw1_hbm.at[:, chunk_cols(c)], sems.at[2]),
                        pltpu.make_async_copy(dw2_st.at[c % 2], dw2_hbm.at[:, chunk_cols(c)], sems.at[3]))

            def hidden_dots(b):
                prod, tails = ((prod_a, tail_a), (prod_b, tail_b))[b % 2]
                mq, kq = FC // np_, DM // np_

                def product(k, lhs, rhs, i, s):
                    v = _dot(lhs.get((i,), 0, mq, slice(None)),
                             rhs.get((i,), 0, kq, cols(s * tg + b * tw, tw)))
                    prod[k, i, s] = v
                    return v

                def tail(k, t):
                    cs = cols(t * tg + b * tw, tw)
                    rem = rem_y.get((), 0, 128, cs) if k == 0 else g_v[pl.ds(DM, 128), cs]
                    v = _dot((rem_pre, rem_dh)[k].get((), 0, FC, slice(None)), rem)
                    tails[k, t] = v
                    return v

                dots = []
                for k, (lhs, rhs) in enumerate(((lhs_pre, rhs_y), (lhs_dh, rhs_g))):
                    dots += [part(product, k, lhs, rhs, i, s) for i in range(rp) for s in range(ng // np_)]
                    dots += [part(tail, k, t) for t in range(ng)]
                return dots

            def pointwise_tasks(b):
                prod, tails = ((prod_a, tail_a), (prod_b, tail_b))[b % 2]
                sub, sub_b, fq = ng // np_, ng // nb_, FC // ng

                def rows_of(r, t, gate):
                    at = r // 32 * 32 + r % 2 * 16 + r // 16 % 2 * 8
                    vals = []
                    for k in range(2):
                        grid = [[None] * ng for _ in range(ng)]
                        for sr in range(sub):
                            for sc in range(sub):
                                m = [prod[k + z, i, sc, pl.ds(sr * fq + at, 8), cols(t)] for i in range(rp)]
                                m = [gate(v) if i % 7 in (0, 2, 3) else v for i, v in enumerate(m)]
                                blk = _collapse(_out_sums, m)
                                for a in range(np_):
                                    for e in range(np_):
                                        fa, te = a * sub + sr, e * sub + sc
                                        grid[fa][te] = blk[a][e] + tails[k + z, te, pl.ds(fa * fq + at, 8), cols(t)]
                        vals.append(grid)
                    hid = [[None] * ng for _ in range(ng)]
                    dpre = [[None] * ng for _ in range(ng)]
                    for a in range(ng):
                        for e in range(ng):
                            hid[a][e], slope = _gelu_and_grad(vals[0][a][e])
                            dpre[a][e] = vals[1][a][e] * slope
                        db1_acc[r % 2, (b * tw + t) // 128, pl.ds((a * fq + r) // 2, 8), :] = _sum(dpre[a])
                    return [[[_expand(_rhs_forms, [[grid[a * sub_b + sr][e * sub_b + sc] for e in range(nb_)]
                                                   for a in range(nb_)])
                              for sc in range(sub_b)] for sr in range(sub_b)] for grid in (hid, dpre)]

                held = []

                def even_rows(r, t, gate):
                    held.append(rows_of(r, t, gate))

                def odd_rows(r, t, gate):
                    even, odd = held.pop(), rows_of(r + 1, t, gate)
                    for k, dst in enumerate((h_st[b], dp_st[b])):
                        for sr in range(sub_b):
                            for sc in range(sub_b):
                                for i in range(rb):
                                    dst.put_pair((i, sc), sr * fq + r, cols(t), even[k][sr][sc][i], odd[k][sr][sc][i])
                return [part(f, r, t) for t in range(0, tw, 128) for r in range(0, fq, 16)
                        for f in (even_rows, odd_rows)]

            def token_dots(b):
                mq, kq = D // nb_, FC // nb_

                def product(lhs, st, acc, i, sc):
                    v = _dot(lhs.get((i + opaque_zero,), 0, mq, slice(None)),
                             st.get((i + opaque_zero, sc), 0, kq, slice(None)))
                    for t in range(0, tw, 128):
                        acc[i, (sc * tg + b * tw + t) // 128] += v[:, t:t + 128]
                    return v
                return [part(product, lhs, st, acc, i, sc)
                        for lhs, st, acc in ((lhs_out, h_st[b], acc_o), (lhs_dy, dp_st[b], acc_y))
                        for i in range(rb) for sc in range(ng // nb_)]

            def weight_grad(cot, st, prods, dst):
                mq, fq, tq = D // nb_, FC // nb_, S // nb_

                blocks = [(sc, b) for sc in range(ng // nb_) for b in range(NB)]
                partial = {}

                def product(i, n, k):
                    rhs = jnp.concatenate([st[b].get((i + opaque_zero, sc), n, 128, slice(None))
                                           for sc, b in blocks[k // tw:(k + 512) // tw]], axis=1)
                    v = _dot(cot.get((i,), 0, mq, cols(k, 512)), rhs, NT)
                    partial[i, n] = v if k == 0 else partial[i, n] + v
                    if k + 512 == tq:
                        prods[i, :, cols(n)] = partial[i, n]
                    return v

                def combine(r, gate):
                    m = [prods[i + z, pl.ds(r, 16), :] for i in range(rb)]
                    blk = _collapse(_lhs_sums, [gate(v) if i % 7 in (0, 1, 4) else v for i, v in enumerate(m)])
                    for a in range(nb_):
                        for e in range(nb_):
                            dst[pl.ds(a * mq + r, 16), pl.ds(e * fq, fq)] = blk[a][e].astype(BF16)
                    return blk[-1][-1]
                return ([part(product, i, n, k) for i in range(rb) for n in range(0, fq, 128)
                         for k in range(0, tq, 512)], [part(combine, r) for r in range(0, mq, 16)])

            def step(c, state):
                nxt, ahead = jnp.minimum(c + 1, NC - 1), jnp.minimum(c + 2, NC - 1)
                for cp in w_copies(nxt, (c + 1) % 3):
                    cp.wait()
                for cp in w_copies(ahead, (c + 2) % 3):
                    cp.start()
                att = attention_tasks(c)
                cut = [len(att) * k // 100 for k in ATT_SPLIT]
                pacer.run(hidden_dots(0), f_stack_tasks(c % 3), att[:cut[0]])
                for b in range(1, NB):
                    pacer.run(hidden_dots(b), pointwise_tasks(b - 1))
                pacer.run(token_dots(0), pointwise_tasks(NB - 1) + [_idle] * IDLE[0])
                dots2, combine2 = weight_grad(cot_g, h_st, wg2, dw2_st.at[c % 2])
                dots1, combine1 = weight_grad(cot_y, dp_st, wg1, dw1_st.at[c % 2])

                def bias1_rows(n, k, gate):
                    db1_tmp[pl.ds(n + k, 8, stride=2), :] = _sum(
                        [gate(db1_acc[k + z, t, pl.ds(n // 2, 8), :]) for t in range(tg // 128)])

                def bias1_grad(n, gate):
                    v = db1_tmp[pl.ds(n, 128), :]
                    v = jnp.concatenate([gate(v[:8]), v[8:]], axis=0).T
                    db1_ref[c, :, cols(n)] = jnp.sum(v, axis=0, keepdims=True).astype(BF16)

                late = [t for b in range(1, NB) for t in token_dots(b)]
                dst = d_stack_tasks(nxt, (c + 1) % 3)
                pacer.run(late[:IDLE[2]], att[cut[0]:cut[1]])
                pacer.run(dots2, att[cut[1]:cut[2]],
                          [part(bias1_rows, n, k) for n in range(0, FC, 16) for k in range(2)]
                          + [part(bias1_grad, n) for n in range(0, FC, 128)] + dst[:len(dst) // 3])
                pacer.run(dots1, att[cut[2]:cut[3]], dst[len(dst) // 3:])
                pacer.run(late[IDLE[2]:], att[cut[3]:] + [_idle] * IDLE[1],
                          combine2 + combine1 + [_idle] * 4)

                @pl.when(c > 0)
                def _():
                    for cp in out_copies(c - 1):
                        cp.wait()

                for cp in out_copies(c):
                    cp.start()
                return state

            carry[...] = jnp.zeros(carry.shape, F32)
            for cp in w_copies(1, 1):
                cp.start()
            lax.fori_loop(0, NC, step, 0)
            for cp in (*w_copies(NC - 1, (NC + 1) % 3), *out_copies(NC - 1)):
                cp.wait()

        mb, kb = D // nb_, FC // nb_
        ng = max(np_, nb_)
        tg = S // ng
        tw = tg // NB
        prod = pltpu.VMEM((2, rp, ng // np_, FC // np_, tw), F32)
        tails = pltpu.VMEM((2, ng, FC, tw), F32)
        pl.run_scoped(
            loop,
            _packed(rb, mb, kb), _packed(rb, mb, kb),
            pltpu.VMEM((2, D, FC), BF16), pltpu.VMEM((2, D, FC), BF16),
            pltpu.VMEM((4, 9, HG, 128), F32), pltpu.VMEM((4, 8, HG, 128), F32),
            pltpu.VMEM((DH, WIN, 8, 128), F32), pltpu.VMEM((DH, WIN, 8, 128), F32),
            pltpu.VMEM((8, WIN, 8, 128), F32), pltpu.VMEM((8, WIN, 8, 128), F32),
            pltpu.VMEM((2, 2, WIN, 8, 128), F32), pltpu.VMEM((2, tg // 128, FC // 2, 128), F32), pltpu.VMEM((FC, 128), F32),
            prod, prod, tails, tails, pltpu.VMEM((rb, mb, kb), F32), pltpu.VMEM((rb, mb, kb), F32),
            *[_packed(rb, ng // nb_, kb, tw)] * (2 * NB))

    mp, kp = FC // np_, DM // np_
    pl.run_scoped(
        main,
        _packed(Q3, S), _packed(D, S),
        _packed(rp, kp, S // np_), _packed(rp, kp, S // np_), _packed(128, S),
        _packed(rb, D // nb_, S // nb_), _packed(rb, D // nb_, S // nb_),
        pltpu.VMEM((3, D, FC), BF16), pltpu.VMEM((3, D, FC), BF16),
        _packed(rp, mp, kp), _packed(rp, mp, kp),
        _packed(FC, 128), _packed(FC, 128), pltpu.VMEM((5, FC, 128), F32))

    def epilogue(branch, out_v, dx_v, dwqkv_v, dwo_v):
        mq, tq = D // nb_, S // nb_
        row = lax.broadcasted_iota(jnp.int32, (DP - D, S), 0)
        o_v.put((), D, slice(None), jnp.where(row == 0, 1.0, 0.0))

        def collapsed(acc, r, t, gate):
            rows = pl.ds(r // 16 * 16 + r // 8 % 2, 8, stride=2)
            blk = _collapse(_out_sums, [gate(acc[i, t, rows, :]) for i in range(rb)])
            return [(pl.ds(a * mq + r, 8), cols(e * tq + t * 128), blk[a][e]) for a in range(nb_) for e in range(nb_)]

        def finish_out(r, t, gate):
            for rows, cs, v in collapsed(acc_o, r, t, gate):
                out_v[rows, cs] = (branch[z, rows, cs] + v).astype(BF16)

        def gather_dy(r, t, gate):
            for rows, cs, v in collapsed(acc_y, r, t, gate):
                branch[1, rows, cs] = v

        def finish_dx(t, gate):
            r1, m2, r2 = (stats[pl.ds(k, 1), cols(t)] for k in range(3))
            xn = xn_v[:, cols(t)]
            y = (xn - m2) * r2
            dy = branch[1 + z, :, cols(t)]
            dy = jnp.concatenate([gate(dy[:8]), dy[8:]], axis=0)
            dxn = branch[2 + z, :, cols(t)] + r2 * (dy - _colmean(dy) - y * _colmean(dy * y))
            dx = r1 * (dxn - _colmean(dxn) - xn * _colmean(dxn * xn))
            dx_v[:, cols(t)] = (g_v[pl.ds(0, D), cols(t)].astype(F32) + dx).astype(BF16)

        def out_dot(t):
            v = _dot(wot.get((), 0, D, slice(None)), o_v.get((), 0, DP, cols(t, 256)))
            branch[0, :, cols(t, 256)] = v + x_v[:, cols(t, 256)].astype(F32)
            return v

        def dxn_dot(t):
            branch[2, :, cols(t, 256)] = v = _dot(wqkv_v[...], dqkv.get((), 0, Q3, cols(t, 256)))
            return v

        def dwqkv_dot(q, n):
            v = _dot(xnb.get((), 0, D, slice(None)), dqkv.get((), q, n, slice(None)), NT)
            dwqkv_v[:, cols(q, n)] = v.astype(BF16)
            return v

        def dwo_dot(r):
            dwo_v[pl.ds(r, 192), :] = _dot(o_v.get((), r, 192, slice(None)), g_v[pl.ds(0, D), :], NT).astype(BF16)

        cp_out = pltpu.make_async_copy(out_v, out_hbm, sems.at[0])
        cp_dx = pltpu.make_async_copy(dx_v, dx_hbm, sems.at[1])
        cp_dwq = pltpu.make_async_copy(dwqkv_v, dwqkv_hbm, sems.at[2])
        cp_dwo = pltpu.make_async_copy(dwo_v, dwo_hbm, sems.at[3])
        for dot, task in ((out_dot, gather_dy), (dxn_dot, finish_out)):
            @pl.loop(0, 4)
            def _(n):
                pacer.run([part(dot, n * 512 + t) for t in (0, 256)],
                          [part(task, r, 2 * n + t) for t in range(2) for r in range(0, mq, 8)])
        cp_out.start()

        @pl.loop(0, 4)
        def _(n):
            pacer.run([part(dwqkv_dot, n * 384 + q, 128) for q in range(0, 384, 128)],
                      [part(finish_dx, n * 512 + t) for t in range(0, 512, 128)] + [_idle] * 2)

        cp_dx.start()
        dwqkv_dot(1536, Q3 - 1536)
        cp_dwq.start()
        for r in range(0, D, 192):
            dwo_dot(r)
        cp_dwo.start()
        for cp in (cp_out, cp_dx, cp_dwq, cp_dwo):
            cp.wait()

    pl.run_scoped(
        epilogue,
        pltpu.VMEM((3, D, S), F32), pltpu.VMEM((D, S), BF16), pltpu.VMEM((D, S), BF16),
        pltpu.VMEM((D, Q3), BF16), pltpu.VMEM((D, D), BF16))


@jax.jit
def pallas_parallel_sum__sliding_local_dilated__mixer_channel_mlp__prompt_kernel(
    A_x: jax.Array,
    A_wqkv: jax.Array,
    A_wo: jax.Array,
    B_x: jax.Array,
    B_w1: jax.Array,
    B_b1: jax.Array,
    B_w2: jax.Array,
    B_b2: jax.Array,
    grad_out: jax.Array,
):
    del B_x
    nb_ = 2 ** LB
    acc = pltpu.VMEM((7 ** LB, S // nb_ // 128, D // nb_, 128), F32)
    hbm = pl.BlockSpec(memory_space=pltpu.HBM)
    vmem = pl.BlockSpec(memory_space=pltpu.VMEM)
    out, dx, dwqkv, dwo, dw1, db1, dw2, db2 = pl.pallas_call(
        _kernel,
        in_specs=[hbm, hbm, hbm, hbm, vmem, hbm, vmem, hbm],
        out_specs=[hbm, hbm, hbm, hbm, hbm, vmem, hbm, vmem],
        out_shape=[
            jax.ShapeDtypeStruct((D, S), BF16), jax.ShapeDtypeStruct((D, S), BF16),
            jax.ShapeDtypeStruct((D, Q3), BF16), jax.ShapeDtypeStruct((D, D), BF16),
            jax.ShapeDtypeStruct((D, F), BF16), jax.ShapeDtypeStruct((NC, 1, FC), BF16),
            jax.ShapeDtypeStruct((D, F), BF16), jax.ShapeDtypeStruct((1, D), BF16),
        ],
        scratch_shapes=[
            pltpu.VMEM((D, S), BF16), pltpu.VMEM((DP, S), BF16),
            pltpu.VMEM((D, S), F32), _packed(DP, S), pltpu.VMEM((8, S), F32),
            _packed(Q3, S), _packed(DP, S),
            pltpu.VMEM((D, Q3), BF16), _packed(D, DP),
            acc, acc,
            pltpu.SemaphoreType.DMA((9,)),
        ],
        compiler_params=pltpu.CompilerParams(vmem_limit_bytes=127 * 2 ** 20),
        name="attn_mlp_fwd_bwd",
    )(A_x.reshape(S, D).T, A_wqkv, A_wo, B_w1, B_b1.reshape(NC, 1, FC), B_w2.T, B_b2.reshape(1, D),
      grad_out.reshape(S, D).T)
    return (out.T.reshape(1, S, D), dx.T.reshape(1, S, D), dwqkv, dwo, dw1, db1.reshape(F), dw2.T,
            db2.reshape(D))
```
